```python
import os as _os
_os.environ.setdefault("JAX_PLATFORMS", "cpu")
import jax
import jax.numpy as jnp

def _softmax(x, axis=-1):
    return jax.nn.softmax(x, axis=axis)
def _gelu(x):
    return jax.nn.gelu(x, approximate=True)
def _silu(x):
    return jax.nn.silu(x)
def _sigmoid(x):
    return jax.nn.sigmoid(x)
def _layernorm(x, axis=-1, eps=1e-5):
    m = jnp.mean(x, axis=axis, keepdims=True)
    v = jnp.var(x, axis=axis, keepdims=True)
    return (x - m) / jnp.sqrt(v + eps)
def _scatter_add(tgt, idx, src, axis=0):
    return tgt.at[idx].add(src)
def _segment_sum(src, seg, n):
    return jax.ops.segment_sum(src, seg, n)
class _Rng:
    def __init__(self, key):
        self._k = key
    def _next(self):
        self._k, sub = jax.random.split(self._k)
        return sub
    def normal(self, shape):
        return jax.random.normal(self._next(), shape, dtype=jnp.bfloat16)
    def randint(self, lo, hi, shape):
        return jax.random.randint(self._next(), shape, lo, hi, dtype=jnp.int32)
    def uniform(self, shape, lo=0.0, hi=1.0):
        return jax.random.uniform(self._next(), shape, jnp.bfloat16, lo, hi)
    def permutation(self, n):
        return jax.random.permutation(self._next(), n)


kernel_name = 'standalone__mha_block_cached__near_ridge'

def setup_inputs():
    _rng = _Rng(jax.random.key(int.from_bytes(__import__("os").urandom(4), "little")))
    _w = (lambda a: (lambda t: t.astype(jnp.bfloat16) if jnp.issubdtype(t.dtype, jnp.floating) else t)(jnp.asarray(a)))
    B, Sq, D = 8, 144, 448
    H, Sk, Dh = 16, 2048, 256
    return {
        "x": _w((lambda *s: _rng.normal(s) * 0.8)(B, Sq, D)),
        "k_cache": _w((lambda *s: _rng.normal(s) * 0.8)(B, H, Sk, Dh)),
        "v_cache": _w((lambda *s: _rng.normal(s) * 0.05)(B, H, Sk, Dh)),
        "wq": _w((lambda *s: _rng.normal(s) * 0.8)(D, H * Dh) * (D ** -0.5)),
        "wo": _w((lambda *s: _rng.normal(s) * 0.05)(H * Dh, D) * ((H * Dh) ** -0.5)),
    }

def reference(x, k_cache, v_cache, wq, wo):
    B, Sq, D = x.shape
    H, Dh = 16, 256
    q = (lambda x, *d: x.transpose(*d))((x @ wq).reshape(B, Sq, H, Dh), 0, 2, 1, 3)
    scores = jnp.einsum("bhqd,bhkd->bhqk", q, k_cache) * (Dh ** -0.5)
    p = _softmax(scores, axis=-1)
    o = jnp.einsum("bhqk,bhkd->bhqd", p, v_cache)
    return (lambda x, *d: x.transpose(*d))(o, 0, 2, 1, 3).reshape(B, Sq, H * Dh) @ wo
```

```python
import functools
import jax
import jax.numpy as jnp
import jax.experimental.pallas as pl
import jax.experimental.pallas.tpu as pltpu

B, SQ, D = 8, 144, 448
H, SK, DH = 16, 2048, 256
LOG2E = 1.4426950408889634
NSTEP = B * H
DEPTH = 4
NHI = 8
SUB = 96
HI_ROWS = NHI * SUB
CH = 256
NCH = SK // CH


def _kernel(x_hbm, k_hbm, v_hbm, wq_hbm, wot_hbm, o_hbm,
            kbuf, vbuf, xbuf, wqbuf, wobuf, acc_ref, obuf,
            ksem, vsem, xsem, wqsem, wosem, osem):
    def lo_copy(hbm, buf, sem, i):
        s = i % DEPTH
        return pltpu.make_async_copy(hbm.at[i, pl.ds(HI_ROWS, SK - HI_ROWS)],
                                     buf.at[s, pl.ds(HI_ROWS, SK - HI_ROWS)], sem.at[s])

    def hi_copy(hbm, buf, sem, i, j):
        s = i % DEPTH
        return pltpu.make_async_copy(hbm.at[i, pl.ds(j * SUB, SUB)],
                                     buf.at[s, pl.ds(j * SUB, SUB)], sem.at[s])

    def all_copy(hbm, buf, sem, i):
        s = i % DEPTH
        return pltpu.make_async_copy(hbm.at[i], buf.at[s], sem.at[s])

    def x_copy(b):
        return pltpu.make_async_copy(x_hbm.at[b], xbuf.at[b % 2], xsem.at[b % 2])

    def wq_copy(h):
        return pltpu.make_async_copy(wq_hbm.at[:, pl.ds(h * DH, DH)], wqbuf.at[h], wqsem.at[h % DEPTH])

    def wo_copy(h):
        return pltpu.make_async_copy(wot_hbm.at[:, pl.ds(h * DH, DH)], wobuf.at[h], wosem.at[h % DEPTH])

    def o_copy(b):
        return pltpu.make_async_copy(obuf.at[b % 2], o_hbm.at[b], osem.at[b % 2])

    x_copy(0).start(priority=1)
    for i in range(DEPTH - 1):
        wq_copy(i).start(priority=1)
        if i < 2:
            all_copy(k_hbm, kbuf, ksem, i).start(priority=1)
            all_copy(v_hbm, vbuf, vsem, i).start(priority=1)
        else:
            lo_copy(k_hbm, kbuf, ksem, i).start(priority=1)
            lo_copy(v_hbm, vbuf, vsem, i).start(priority=1)
        wo_copy(i).start(priority=1)

    def step(i, carry):
        b = i // H
        h = i % H
        s = i % DEPTH
        ia = i + DEPTH - 1

        @pl.when(ia < NSTEP)
        def _():
            @pl.when(ia % H == 0)
            def _():
                x_copy(ia // H).start(priority=1)
            @pl.when(ia < H)
            def _():
                wq_copy(ia).start(priority=1)
            lo_copy(k_hbm, kbuf, ksem, ia).start(priority=1)
            lo_copy(v_hbm, vbuf, vsem, ia).start(priority=1)
            @pl.when(ia < H)
            def _():
                wo_copy(ia).start(priority=1)

        @pl.when(h == 0)
        def _():
            x_copy(b).wait()

        @pl.when(i < H)
        def _():
            wq_copy(i).wait()
            wo_copy(i).wait()

        all_copy(k_hbm, kbuf, ksem, i).wait()
        all_copy(v_hbm, vbuf, vsem, i).wait()

        do_hi = i + 2 < NSTEP
        nxt = jnp.minimum(i + 2, NSTEP - 1)

        def hi(hbm, buf, sem, j):
            @pl.when(do_hi)
            def _():
                hi_copy(hbm, buf, sem, nxt, j).start(priority=0)

        q = jnp.dot(xbuf[b % 2], wqbuf[h], preferred_element_type=jnp.float32)
        q = (q * (DH ** -0.5 * LOG2E)).astype(jnp.bfloat16)
        ss = []
        for c in range(NCH):
            hi(k_hbm, kbuf, ksem, c)
            kc = kbuf[s, pl.ds(c * CH, CH), :]
            ss.append(jax.lax.dot_general(q, kc, (((1,), (1,)), ((), ())), preferred_element_type=jnp.float32))
        mm = ss[0]
        for c in range(1, NCH):
            mm = jnp.maximum(mm, ss[c])
        m = jnp.max(mm, axis=-1, keepdims=True)
        lacc = None
        o = None
        for c in range(NCH):
            hi(v_hbm, vbuf, vsem, c)
            p = jnp.exp2(ss[c] - m)
            lacc = p if lacc is None else lacc + p
            vc = vbuf[s, pl.ds(c * CH, CH), :]
            pv = jnp.dot(p.astype(jnp.bfloat16), vc, preferred_element_type=jnp.float32)
            o = pv if o is None else o + pv
        l = jnp.sum(lacc, axis=-1, keepdims=True)
        o = (o / l).astype(jnp.bfloat16)
        y = jax.lax.dot_general(o, wobuf[h], (((1,), (1,)), ((), ())), preferred_element_type=jnp.float32)

        @pl.when(h == 0)
        def _():
            acc_ref[...] = y

        @pl.when(h > 0)
        def _():
            acc_ref[...] += y

        @pl.when(h == H - 1)
        def _():
            @pl.when(b >= 2)
            def _():
                o_copy(b - 2).wait()
            obuf[b % 2] = acc_ref[...].astype(obuf.dtype)
            o_copy(b).start()
        return carry

    jax.lax.fori_loop(0, NSTEP, step, 0)
    o_copy(B - 2).wait()
    o_copy(B - 1).wait()


@jax.jit
def pallas_standalone__mha_block_cached__near_ridge_kernel(x, k_cache, v_cache, wq, wo):
    k3 = k_cache.reshape(NSTEP, SK, DH)
    v3 = v_cache.reshape(NSTEP, SK, DH)
    wot = wo.T
    any_spec = pl.BlockSpec(memory_space=pl.ANY)
    bf = jnp.bfloat16
    return pl.pallas_call(
        _kernel,
        in_specs=[any_spec] * 5,
        out_specs=any_spec,
        out_shape=jax.ShapeDtypeStruct((B, SQ, D), x.dtype),
        scratch_shapes=[
            pltpu.VMEM((DEPTH, SK, DH), bf),
            pltpu.VMEM((DEPTH, SK, DH), bf),
            pltpu.VMEM((2, SQ, D), bf),
            pltpu.VMEM((H, D, DH), bf),
            pltpu.VMEM((H, D, DH), bf),
            pltpu.VMEM((SQ, D), jnp.float32),
            pltpu.VMEM((2, SQ, D), bf),
            pltpu.SemaphoreType.DMA((DEPTH,)),
            pltpu.SemaphoreType.DMA((DEPTH,)),
            pltpu.SemaphoreType.DMA((2,)),
            pltpu.SemaphoreType.DMA((DEPTH,)),
            pltpu.SemaphoreType.DMA((DEPTH,)),
            pltpu.SemaphoreType.DMA((2,)),
        ],
        compiler_params=pltpu.CompilerParams(
            vmem_limit_bytes=64 * 1024 * 1024,
            disable_bounds_checks=True,
            disable_semaphore_checks=True,
        ),
    )(x, k3, v3, wq, wot)
```

```python
import functools
import os
import jax
import jax.numpy as jnp
import jax.experimental.pallas as pl
import jax.experimental.pallas.tpu as pltpu

B, SQ, D = 8, 144, 448
H, SK, DH = 16, 2048, 256
LOG2E = 1.4426950408889634
NSTEP = B * H
T = 128
NT = SK // T
NS = int(os.environ.get("NS", 4))
DEPTH = 8 if NS == 4 else 16
PR = SK // NS
TP = NT // NS
NP = int(os.environ.get("NP", 22))
P0 = int(os.environ.get("P0", 7))
WP = int(os.environ.get("WP", 4))
SKEW = int(os.environ.get("SKEW", 2))
USTAR = int(os.environ.get("USTAR", 117))
UPC = int(os.environ.get("UPC", 6))
FULLN = int(os.environ.get("FULLN", 2))
XN = int(os.environ.get("XN", 0))
KADV = int(os.environ.get("KADV", 2))
INNER = int(os.environ.get("INNER", 1))
TA = 12
SCOPES = int(os.environ.get("SCOPES", 0))
NT_DIMS = (((1,), (1,)), ((), ()))
HI, LO = 0, 1
BF = jnp.bfloat16
F32 = jnp.float32


def _spread(total, m, g=8):
    units = total // g
    out, o = [], 0
    for j in range(m):
        e = ((j + 1) * units) // m * g
        out.append((o, e - o))
        o = e
    return out

PIECES = _spread(PR, NP)
WPIECES = _spread(D, WP)
KS, VS, WQS, WOS, XS, OS, VB = 0, DEPTH, 2 * DEPTH, 2 * DEPTH + 4, 2 * DEPTH + 8, 2 * DEPTH + 10, 2 * DEPTH + 12
NSEM = VB + 1


def _plain_stream():
    upc = max(1, UPC * PR // 512)
    sub = _spread(PR, upc)
    out = []
    for j in range(USTAR + 1, NSTEP):
        rs = [r for r in range(NS) if j - r > USTAR]
        if INNER and len(rs) == NS and j != NSTEP - 2:
            for r in range(NS // 2):
                for o, n in sub:
                    out.append((j, r, o, n))
                    out.append((j, r + NS // 2, o, n))
        else:
            for r in rs:
                for o, n in sub:
                    out.append((j, r, o, n))
    return out

PLAIN = _plain_stream()
W0 = USTAR - 2


def _plain_counts():
    per_slab = len([1 for p in PLAIN if p[0] == NSTEP - 1])
    steps = list(range(W0, NSTEP - 2))
    cnt = {W0: P0 * per_slab // NP}
    for s in steps[1:1 + FULLN]:
        cnt[s] = per_slab
    rest = steps[1 + FULLN:]
    left = len(PLAIN) - sum(cnt.values()) - XN
    for n, s in enumerate(rest):
        cnt[s] = ((n + 1) * left) // len(rest) - (n * left) // len(rest)
    pos, out = 0, {}
    for s in steps:
        out[s] = (pos, pos + cnt[s])
        pos += cnt[s]
    out[NSTEP - 2] = (pos, len(PLAIN))
    return out

PCNT = _plain_counts()


def _wait(name, *copies):
    if SCOPES:
        with jax.named_scope(name):
            for c in copies:
                c.wait()
    else:
        for c in copies:
            c.wait()


def _kernel(x_hbm, k_hbm, v_hbm, wq_hbm, wot_hbm, o_hbm,
            kbuf, vbuf, xbuf, wqbuf, wobuf, sbuf, mbuf, qbuf, acc_ref, obuf, pbuf, sem):
    K = (k_hbm, kbuf, KS)
    V = (v_hbm, vbuf, VS)
    WQ = (wq_hbm, wqbuf, WQS)
    WO = (wot_hbm, wobuf, WOS)

    def burst_piece(hbm, buf, s0, u, o, r):
        s = u % DEPTH
        row = (u % NS) * PR + o
        if not isinstance(u, int):
            row = pl.multiple_of(row, 8)
        return pltpu.make_async_copy(hbm.at[pl.ds(u, NS), pl.ds(row, r)], buf.at[s, :, pl.ds(o, r)], sem.at[s0 + s])

    def start_burst(u, ps):
        for p in ps:
            burst_piece(*V, u, *PIECES[p]).start(priority=LO)
            burst_piece(*K, u, *PIECES[p]).start(priority=HI)

    def tri_piece(hbm, buf, s0, u, o, r):
        s = u % DEPTH
        return pltpu.make_async_copy(hbm.at[pl.ds(0, NS + u), pl.ds((u % NS) * PR + o, r)],
                                     buf.at[s, pl.ds(-u, NS + u), pl.ds(o, r)], sem.at[s0 + s])

    def units(buf, si, n):
        return pltpu.make_async_copy(buf.at[0, pl.ds(0, n)], buf.at[0, pl.ds(0, n)], sem.at[si])

    def plain_piece(hbm, buf, s0, j, r, o, n):
        si = s0 + j % DEPTH
        if s0 == VS and j == NSTEP - 2 and r * TP >= TA:
            si = VB
        return pltpu.make_async_copy(hbm.at[j, pl.ds(((j - r) % NS) * PR + o, n)],
                                     buf.at[(j - r) % DEPTH, r, pl.ds(o, n)], sem.at[si])

    def start_plain(a, b, kadv=0, kskip=0):
        vs = list(range(a, b))
        ks = list(range(a + kskip, min(b + kadv, len(PLAIN)))) if True else []
        n = len(vs)
        for t in range(n):
            plain_piece(*V, *PLAIN[vs[t]]).start(priority=LO)
            if ks:
                plain_piece(*K, *PLAIN[ks.pop(0)]).start(priority=HI)
        while ks:
            plain_piece(*K, *PLAIN[ks.pop(0)]).start(priority=HI)

    def nunits(j):
        return min(NS, j - USTAR) if j > USTAR else NS

    def x_copy(b):
        return pltpu.make_async_copy(x_hbm.at[b], xbuf.at[b % 2], sem.at[XS + b % 2])

    def w_piece(hbm, buf, s0, h, p):
        o, r = WPIECES[p]
        return pltpu.make_async_copy(hbm.at[pl.ds(o, r), pl.ds(h * DH, DH)], buf.at[h, pl.ds(o, r)],
                                     sem.at[s0 + h % 4])

    def w_all(hbm, buf, s0, h):
        return pltpu.make_async_copy(hbm.at[:, pl.ds(h * DH, DH)], buf.at[h], sem.at[s0 + h % 4])

    def o_copy(b0, n, s):
        return pltpu.make_async_copy(obuf.at[pl.ds(b0, n)], o_hbm.at[pl.ds(b0, n)], sem.at[OS + s])

    def start_w(ho, hq):
        for p in range(WP):
            if ho is not None:
                w_piece(*WO, ho, p).start(priority=LO)
            if hq is not None:
                w_piece(*WQ, hq, p).start(priority=HI)

    x_copy(0).start(priority=HI)
    start_w(None, 0)
    start_w(0, 1)
    for u in range(1 - NS, 0):
        for o, r in _spread(PR, max(1, (NP * (NS + u) + NS - 1) // NS)):
            tri_piece(*V, u, o, r).start(priority=LO)
            tri_piece(*K, u, o, r).start(priority=HI)
    start_burst(0, range(NP))
    start_w(1, 2)
    start_burst(1, range(NP))
    start_w(2, 3)
    start_burst(2, range(P0))
    acc_ref[...] = jnp.zeros_like(acc_ref)

    def qproj(i):
        q = jnp.dot(xbuf[(i // H) % 2], wqbuf[i % H], preferred_element_type=F32)
        return (q * (DH ** -0.5 * LOG2E)).astype(BF)

    def cols(c):
        return slice(c * T, (c + 1) * T)

    def kv_tile(buf, j, c):
        r = c // TP
        return buf[(j + DEPTH - r) % DEPTH, r, pl.ds((c % TP) * T, T), :]

    def qk_tile(st, q, i, c):
        s = jax.lax.dot_general(q, kv_tile(kbuf, i, c), NT_DIMS, preferred_element_type=F32)
        sbuf[:, cols(c)] = s
        st["mx"] = s if c == 0 else jnp.maximum(st["mx"], s)

    def row_max(st):
        return jnp.broadcast_to(jnp.max(st["mx"], axis=-1, keepdims=True), (SQ, T))

    def exp_tile(st, m, c):
        p = jnp.exp2(sbuf[:, cols(c)] - m)
        st["l"] = p if c == 0 else st["l"] + p
        return p.astype(BF)

    def inv_sum(st):
        return pl.reciprocal(jnp.sum(st["l"], axis=-1, keepdims=True), approx=False)

    def pv_tile(st, p, i, c):
        pv = jnp.dot(p, kv_tile(vbuf, i, c), preferred_element_type=F32)
        st["o"] = pv if c == 0 else st["o"] + pv

    def onorm(st, rinv):
        return (st["o"] * rinv).astype(BF)

    def oproj(o, i):
        return jax.lax.dot_general(o, wobuf[i % H], NT_DIMS, preferred_element_type=F32)

    _wait("w0", x_copy(0), w_all(*WQ, 0), w_all(*WQ, 1),
          *[units(kbuf, KS + u % DEPTH, NS + u) for u in range(1 - NS, 1)])
    st0 = {}
    q0 = qproj(0)
    qbuf[...] = qproj(1)
    for c in range(NT):
        qk_tile(st0, q0, 0, c)
    mbuf[...] = row_max(st0)

    def step(i, carry):
        @pl.when(i < W0)
        def _():
            start_burst(i + 2, range(P0, NP))

            @pl.when(i + 4 < H)
            def _():
                start_w(i + 3, i + 4)

            @pl.when(i + 4 == H)
            def _():
                start_w(H - 1, None)

            @pl.when((i + 4) % H == 0)
            def _():
                x_copy((i + 4) // H).start(priority=HI)
            start_burst(i + 3, range(P0))

            @pl.when((i + 2) % H == 0)
            def _():
                x_copy((i + 2) // H).wait()

            @pl.when(i + 2 < H)
            def _():
                w_all(*WQ, i + 2).wait()

            @pl.when(i < H)
            def _():
                w_all(*WO, i).wait()

            @pl.when(i == 0)
            def _():
                for u in range(1 - NS, 0):
                    units(vbuf, VS + u % DEPTH, NS + u).wait()

            _wait("wK", units(kbuf, KS + (i + 1) % DEPTH, NS))
            _wait("wV", units(vbuf, VS + i % DEPTH, NS))

        @pl.when(i >= W0)
        def _():
            for s in range(W0, NSTEP - 2):
                @pl.when(i == s)
                def _(s=s):
                    if s == W0:
                        start_burst(USTAR, range(P0, NP))
                    last = s == NSTEP - 3
                    start_plain(*PCNT[s], kadv=len(PLAIN) if last else (KADV if s == NSTEP - 4 else 0),
                                kskip=KADV if last else 0)
                    _wait("wK", units(kbuf, KS + (s + 1) % DEPTH, nunits(s + 1)))
                    _wait("wV", units(vbuf, VS + s % DEPTH, nunits(s)))

        st = {}
        m = mbuf[...]
        q = qbuf[...]
        for c in range(NT + SKEW):
            if c < NT:
                pv_tile(st, exp_tile(st, m, c), i, c)
            if c == 0:
                qn = qproj(i + 2)
            if c >= SKEW:
                qk_tile(st, q, i + 1, c - SKEW)
        acc_ref[...] += oproj(onorm(st, inv_sum(st)), i)
        qbuf[...] = qn
        mbuf[...] = row_max(st)

        @pl.when(i % H == H - 1)
        def _():
            obuf[i // H] = acc_ref[...].astype(BF)
            acc_ref[...] = jnp.zeros_like(acc_ref)
        return carry

    jax.lax.fori_loop(0, NSTEP - 2, step, 0)

    i1, i2 = NSTEP - 2, NSTEP - 1
    for t in range(*PCNT[i1]):
        plain_piece(*V, *PLAIN[t]).start(priority=LO)
    _wait("wKx", units(kbuf, KS + i2 % DEPTH, NS))
    _wait("wVx", units(vbuf, VS + i1 % DEPTH, TA // TP))
    s1, s2 = {}, {}
    m = mbuf[...]
    q = qbuf[...]
    for c in range(NT):
        p = exp_tile(s1, m, c)
        if c < TA:
            pv_tile(s1, p, i1, c)
        else:
            pbuf[:, cols(c - TA)] = p
        qk_tile(s2, q, i2, c)
    r1 = inv_sum(s1)
    m2 = row_max(s2)
    _wait("wVz", units(vbuf, VB, NS - TA // TP), units(vbuf, VS + i2 % DEPTH, NS))
    o_copy(0, B - 1, 0).start(priority=LO)
    for c in range(TA, NT):
        pv_tile(s1, pbuf[:, cols(c - TA)], i1, c)
    o1 = onorm(s1, r1)
    for c in range(NT):
        pv_tile(s2, exp_tile(s2, m2, c), i2, c)
    y1 = acc_ref[...] + oproj(o1, i1)
    obuf[B - 1] = (y1 + oproj(onorm(s2, inv_sum(s2)), i2)).astype(BF)
    o_copy(B - 1, 1, 1).start(priority=HI)
    _wait("wO1", o_copy(0, B - 1, 0))
    _wait("wO2", o_copy(B - 1, 1, 1))


@jax.jit
def pallas_standalone__mha_block_cached__near_ridge_kernel(x, k_cache, v_cache, wq, wo):
    k3 = k_cache.reshape(NSTEP, SK, DH)
    v3 = v_cache.reshape(NSTEP, SK, DH)
    wot = wo.T
    any_spec = pl.BlockSpec(memory_space=pl.ANY)
    return pl.pallas_call(
        _kernel,
        in_specs=[any_spec] * 5,
        out_specs=any_spec,
        out_shape=jax.ShapeDtypeStruct((B, SQ, D), x.dtype),
        scratch_shapes=[
            pltpu.VMEM((DEPTH, NS, PR, DH), BF),
            pltpu.VMEM((DEPTH, NS, PR, DH), BF),
            pltpu.VMEM((2, SQ, D), BF),
            pltpu.VMEM((H, D, DH), BF),
            pltpu.VMEM((H, D, DH), BF),
            pltpu.VMEM((SQ, SK), F32),
            pltpu.VMEM((SQ, T), F32),
            pltpu.VMEM((SQ, DH), BF),
            pltpu.VMEM((SQ, D), F32),
            pltpu.VMEM((B, SQ, D), BF),
            pltpu.VMEM((SQ, (NT - TA) * T), BF),
            pltpu.SemaphoreType.DMA((NSEM,)),
        ],
        compiler_params=pltpu.CompilerParams(
            vmem_limit_bytes=96 * 1024 * 1024,
            disable_bounds_checks=True,
            disable_semaphore_checks=True,
        ),
    )(x, k3, v3, wq, wot)
```

```python
import jax
import jax.numpy as jnp
import jax.experimental.pallas as pl
import jax.experimental.pallas.tpu as pltpu

B, SQ, D = 8, 144, 448
H, SK, DH = 16, 2048, 256
NSTEP = B * H
LOG2E = 1.4426950408889634

T = 128
NT = SK // T
SKEW = 2
TA = 12

NS = 8
PR = SK // NS
TP = NT // NS
DEPTH = 16
NP = 26
P0 = 3
USTAR = 103
W0 = USTAR - 2
AH = 54
KADV = 6
TGT = 88

WG, WC = 4, 6
WR = D // WG
XG, XP = 2, 26
XR = B * SQ // XG

HI, LO = 0, 1
NT_DIMS = (((1,), (1,)), ((), ()))
BF = jnp.bfloat16
F32 = jnp.float32

KS, VS = 0, DEPTH
WQS, WOS, XS, OS0, OS1, VB = range(2 * DEPTH, 2 * DEPTH + 6)
NSEM = VB + 1


def _spread(total, m, g=8):
    units = total // g
    out, o = [], 0
    for j in range(m):
        e = ((j + 1) * units) // m * g
        out.append((o, e - o))
        o = e
    return out


def _merge(lists):
    keyed = [((t + 0.5) / len(l), k, p) for k, l in enumerate(lists) for t, p in enumerate(l)]
    return [p for _, _, p in sorted(keyed)]


def _group_pieces(owner, u, ra, g):
    m = max(1, min(PR // 8, round(g * PR / TGT)))
    return [(owner, u, ra, g, o, n) for o, n in _spread(PR, m)]


def _winddown():
    rem = {(j, r) for j in range(USTAR + 1, NSTEP) for r in range(NS) if j - r > USTAR}
    last_free = NSTEP - 3
    tot = sum(1 for j, _ in rem if j <= last_free)
    budget = {s: tot * (s - USTAR) / (last_free - USTAR) for s in range(USTAR + 1, last_free + 1)}
    cum = 0
    pieces, ends, owned = [], {}, {}
    for s in range(USTAR + 1, NSTEP):
        groups = {r: 1 for j, r in sorted(rem) if j == s}
        rem -= {(s, r) for r in groups}
        cum += len(groups)

        def fits(cand):
            for s2 in range(s, cand[-1][0]):
                need = sum(1 for c in rem if s < c[0] <= s2 and c not in cand)
                if cum + len(cand) + need > budget[s2] + 1e-9:
                    return False
            return True

        grown = s < last_free
        while grown:
            grown = False
            for r in sorted(groups, key=lambda r: (groups[r], r)):
                g = groups[r]
                cand = [(s + g + e, r + g + e) for e in range(2 if g == 6 else 1)]
                if all(c in rem and c[0] <= last_free for c in cand) and fits(cand):
                    rem -= set(cand)
                    cum += len(cand)
                    groups[r] += len(cand)
                    grown = True
                    break

        late = lambda r: s == NSTEP - 2 and r * TP >= TA
        done = set()
        for r in sorted(groups):
            if r in done:
                continue
            mate = r + NS // 2
            both = [r]
            if mate in groups and max(groups[r], groups[mate]) <= 2 and late(r) == late(mate):
                both.append(mate)
            done.update(both)
            pieces += _merge([_group_pieces(s, s - q, q, groups[q]) for q in both])
        ends[s] = len(pieces)
        owned[s] = [(s - r, r, g) for r, g in sorted(groups.items())]
    assert not rem

    ranges, pos = {}, 0
    for s in range(W0, NSTEP - 2):
        end = ends[s] if s > USTAR else (s - USTAR) * NP
        nxt = max(pos, min(len(pieces), end + AH))
        ranges[s] = (pos, nxt)
        pos = nxt
        assert s < USTAR or nxt >= ends[s + 1]
        for owner, u, ra, g, _, _ in pieces[ranges[s][0]:nxt + KADV]:
            assert u + ra + g - 1 - DEPTH < s - 1 and owner - DEPTH < s - 1
    assert pos == len(pieces)
    return pieces, ranges, owned


PIECES = _spread(PR, NP)
WD, WD_RANGE, WD_OWNED = _winddown()
HEAD_GROUPS = {u: ([(u, -u, 4), (u, 4 - u, 3)] if NS + u == 7 else [(u, -u, NS + u)]) for u in range(1 - NS, 0)}


def _owned(j):
    return WD_OWNED[j] if j > USTAR else [(j, 0, NS)]


def _kernel(x_hbm, k_hbm, v_hbm, wq_hbm, wot_hbm, o_hbm,
            kbuf, vbuf, xbuf, wqbuf, wobuf, sbuf, mbuf, qbuf, acc_ref, obuf, pbuf, sem):
    K = (k_hbm, kbuf, KS)
    V = (v_hbm, vbuf, VS)

    def sem_of(s0, owner, ra):
        if s0 == VS and isinstance(owner, int) and owner == NSTEP - 2 and ra * TP >= TA:
            return sem.at[VB]
        return sem.at[s0 + owner % DEPTH]

    def kv_copy(hbm, buf, s0, owner, u, ra, g, o, n):
        row = (u % NS) * PR + o
        if not isinstance(u, int):
            row = pl.multiple_of(row, 8)
        return pltpu.make_async_copy(hbm.at[pl.ds(u + ra, g), pl.ds(row, n)],
                                     buf.at[u % DEPTH, pl.ds(ra, g), pl.ds(o, n)], sem_of(s0, owner, ra))

    def start_pairs(vs, ks):
        for t in range(max(len(vs), len(ks))):
            if t < len(vs):
                kv_copy(*V, *vs[t]).start(priority=LO)
            if t < len(ks):
                kv_copy(*K, *ks[t]).start(priority=HI)

    def start_burst(u, lo, hi):
        ps = [(u, u, 0, NS, o, n) for o, n in PIECES[lo:hi]]
        start_pairs(ps, ps)

    def wait_groups(hbm, buf, s0, owner, groups):
        for u, ra, g in groups:
            dst = buf.at[u % DEPTH, pl.ds(ra, g)]
            pltpu.make_async_copy(dst, dst, sem_of(s0, owner, ra)).wait()

    def w_copy(hbm, buf, si, r, o, n):
        return pltpu.make_async_copy(hbm.at[:, pl.ds(r, 8), pl.ds(o, n)],
                                     buf.at[:, pl.ds(r, 8), pl.ds(o, n)], sem.at[si])

    def o_copy(b0, n, si):
        return pltpu.make_async_copy(obuf.at[pl.ds(b0, n)], o_hbm.at[pl.ds(b0, n)], sem.at[si])

    def w_head(buf, i):
        off = (i % H) * DH
        if not isinstance(i, int):
            off = pl.multiple_of(off, DH)
        return buf[:, :, pl.ds(off, DH)].reshape(D, DH)

    def qproj(i):
        b = i // H
        row = (b % (B // XG)) * SQ
        if not isinstance(i, int):
            row = pl.multiple_of(row, 16)
        q = jnp.dot(xbuf[b // (B // XG), pl.ds(row, SQ), :], w_head(wqbuf, i), preferred_element_type=F32)
        return (q * (DH ** -0.5 * LOG2E)).astype(BF)

    def cols(c):
        return slice(c * T, (c + 1) * T)

    def kv_tile(buf, j, c):
        r = c // TP
        return buf[(j + DEPTH - r) % DEPTH, r, pl.ds((c % TP) * T, T), :]

    def qk_tile(st, q, j, c):
        s = jax.lax.dot_general(q, kv_tile(kbuf, j, c), NT_DIMS, preferred_element_type=F32)
        sbuf[:, cols(c)] = s
        st["mx"] = s if c == 0 else jnp.maximum(st["mx"], s)

    def row_max(st):
        return jnp.broadcast_to(jnp.max(st["mx"], axis=-1, keepdims=True), (SQ, T))

    def exp_tile(st, m, c):
        p = jnp.exp2(sbuf[:, cols(c)] - m)
        st["l"] = p if c == 0 else st["l"] + p
        return p.astype(BF)

    def inv_sum(st):
        return pl.reciprocal(jnp.sum(st["l"], axis=-1, keepdims=True), approx=False)

    def pv_tile(st, p, j, c):
        pv = jnp.dot(p, kv_tile(vbuf, j, c), preferred_element_type=F32)
        st["o"] = pv if c == 0 else st["o"] + pv

    def oproj(st, rinv, j):
        o = (st["o"] * rinv).astype(BF)
        return jax.lax.dot_general(o, w_head(wobuf, j), NT_DIMS, preferred_element_type=F32)

    for o, n in _spread(XR, XP):
        pltpu.make_async_copy(x_hbm.at[:, pl.ds(o, n)], xbuf.at[:, pl.ds(o, n)], sem.at[XS]).start(priority=LO)
    for r in range(0, WR, 8):
        for o, n in _spread(H * DH, WC, 128):
            w_copy(wot_hbm, wobuf, WOS, r, o, n).start(priority=LO)
            w_copy(wq_hbm, wqbuf, WQS, r, o, n).start(priority=HI)
    for u, groups in HEAD_GROUPS.items():
        ps = _merge([_group_pieces(u, *grp) for grp in groups])
        start_pairs(ps, ps)
    start_burst(0, 0, NP)
    start_burst(1, 0, NP)
    start_burst(2, 0, P0)
    acc_ref[...] = jnp.zeros_like(acc_ref)

    pltpu.make_async_copy(x_hbm, xbuf, sem.at[XS]).wait()
    pltpu.make_async_copy(wq_hbm, wqbuf, sem.at[WQS]).wait()
    pltpu.make_async_copy(wot_hbm, wobuf, sem.at[WOS]).wait()
    for u, groups in HEAD_GROUPS.items():
        wait_groups(*K, u, groups)
    wait_groups(*K, 0, _owned(0))
    st0 = {}
    q0 = qproj(0)
    qbuf[...] = qproj(1)
    for c in range(NT):
        qk_tile(st0, q0, 0, c)
    mbuf[...] = row_max(st0)

    def step(i, carry):
        @pl.when(i < W0)
        def _():
            start_burst(i + 2, P0, NP)
            start_burst(i + 3, 0, P0)

            @pl.when(i == 0)
            def _():
                for u, groups in HEAD_GROUPS.items():
                    wait_groups(*V, u, groups)

            wait_groups(*K, i + 1, [(i + 1, 0, NS)])
            wait_groups(*V, i, [(i, 0, NS)])

        def special(s):
            if s == W0:
                start_burst(USTAR, P0, NP)
            lo, hi = WD_RANGE[s]
            klo = lo + (KADV if s == NSTEP - 3 else 0)
            khi = hi + (KADV if s == NSTEP - 4 else 0)
            start_pairs(WD[lo:hi], WD[klo:khi])
            wait_groups(*K, s + 1, _owned(s + 1))
            wait_groups(*V, s, _owned(s))

        def dispatch(lo, hi):
            if hi - lo == 1:
                special(lo)
            else:
                mid = (lo + hi) // 2
                jax.lax.cond(i < mid, lambda: dispatch(lo, mid), lambda: dispatch(mid, hi))

        @pl.when(i >= W0)
        def _():
            dispatch(W0, NSTEP - 2)

        st = {}
        m = mbuf[...]
        q = qbuf[...]
        for c in range(NT + SKEW):
            if c < NT:
                pv_tile(st, exp_tile(st, m, c), i, c)
            if c == 0:
                q_next = qproj(i + 2)
            if c >= SKEW:
                qk_tile(st, q, i + 1, c - SKEW)
        acc_ref[...] += oproj(st, inv_sum(st), i)
        qbuf[...] = q_next
        mbuf[...] = row_max(st)

        @pl.when(i % H == H - 1)
        def _():
            obuf[i // H] = acc_ref[...].astype(BF)
            acc_ref[...] = jnp.zeros_like(acc_ref)
        return carry

    jax.lax.fori_loop(0, NSTEP - 2, step, 0)

    i1, i2 = NSTEP - 2, NSTEP - 1
    wait_groups(*K, i2, _owned(i2))
    wait_groups(*V, i1, [grp for grp in _owned(i1) if grp[1] * TP < TA])
    s1, s2 = {}, {}
    m = mbuf[...]
    q = qbuf[...]
    for c in range(NT):
        p = exp_tile(s1, m, c)
        if c < TA:
            pv_tile(s1, p, i1, c)
        else:
            pbuf[:, cols(c - TA)] = p
        qk_tile(s2, q, i2, c)
    r1 = inv_sum(s1)
    m2 = row_max(s2)

    wait_groups(*V, i2, _owned(i2))
    o_copy(0, B - 1, OS0).start(priority=LO)
    wait_groups(*V, i1, [grp for grp in _owned(i1) if grp[1] * TP >= TA])
    for c in range(TA, NT):
        pv_tile(s1, pbuf[:, cols(c - TA)], i1, c)
    for c in range(NT):
        pv_tile(s2, exp_tile(s2, m2, c), i2, c)
    y = acc_ref[...] + oproj(s1, r1, i1)
    obuf[B - 1] = (y + oproj(s2, inv_sum(s2), i2)).astype(BF)
    o_copy(B - 1, 1, OS1).start(priority=HI)
    o_copy(0, B - 1, OS0).wait()
    o_copy(B - 1, 1, OS1).wait()


@jax.jit
def pallas_standalone__mha_block_cached__near_ridge_kernel(
    x: jax.Array,
    k_cache: jax.Array,
    v_cache: jax.Array,
    wq: jax.Array,
    wo: jax.Array,
):
    any_spec = pl.BlockSpec(memory_space=pl.ANY)
    return pl.pallas_call(
        _kernel,
        in_specs=[any_spec] * 5,
        out_specs=any_spec,
        out_shape=jax.ShapeDtypeStruct((B, SQ, D), x.dtype),
        scratch_shapes=[
            pltpu.VMEM((DEPTH, NS, PR, DH), BF),
            pltpu.VMEM((DEPTH, NS, PR, DH), BF),
            pltpu.VMEM((XG, XR, D), BF),
            pltpu.VMEM((WG, WR, H * DH), BF),
            pltpu.VMEM((WG, WR, H * DH), BF),
            pltpu.VMEM((SQ, SK), F32),
            pltpu.VMEM((SQ, T), F32),
            pltpu.VMEM((SQ, DH), BF),
            pltpu.VMEM((SQ, D), F32),
            pltpu.VMEM((B, SQ, D), BF),
            pltpu.VMEM((SQ, (NT - TA) * T), BF),
            pltpu.SemaphoreType.DMA((NSEM,)),
        ],
        compiler_params=pltpu.CompilerParams(
            vmem_limit_bytes=64 * 1024 * 1024,
            disable_bounds_checks=True,
            disable_semaphore_checks=True,
        ),
    )(
        x.reshape(XG, XR, D),
        k_cache.reshape(NSTEP, SK, DH),
        v_cache.reshape(NSTEP, SK, DH),
        wq.reshape(WG, WR, H * DH),
        wo.T.reshape(WG, WR, H * DH),
    )
```

```python
import jax
import jax.numpy as jnp
import jax.experimental.pallas as pl
import jax.experimental.pallas.tpu as pltpu

B, SQ, D = 8, 144, 448
H, SK, DH = 16, 2048, 256
NSTEP = B * H
LOG2E = 1.4426950408889634

T = 128
NT = SK // T
SKEW = 2

NS = 8
PR = SK // NS
TP = NT // NS
DEPTH = 16
NP = 26
PV0, PK0 = 3, 4
PK = NS - 1
USTAR = 110
W0 = USTAR - 2
NQ = NSTEP - 1 - W0
AH = 54
TGT = 88
I0, I1, I2 = NSTEP - 3, NSTEP - 2, NSTEP - 1
TA = 12
KLO, VHI = 9, 11
ADVS = 122

WG, WC = 4, 6
WR = D // WG
XG, XP = 2, 26
XR = B * SQ // XG
QCH, Q1, QG = 3, 28, 20

HI, LO = 0, 1
NT_DIMS = (((1,), (1,)), ((), ()))
BF = jnp.bfloat16
F32 = jnp.float32

KS, VS = 0, DEPTH
WQS, WOS, XS, OS0, OS1, VL0, VL2 = range(2 * DEPTH, 2 * DEPTH + 7)
NSEM = VL2 + 1


def _late(j, r):
    return (j == I0 and r * TP >= TA) or (j == I2 and r % (NS // 2) == NS // 2 - 1)


def _spread(total, m, g=8):
    units = total // g
    out, o = [], 0
    for j in range(m):
        e = ((j + 1) * units) // m * g
        out.append((o, e - o))
        o = e
    return out


def _merge(lists):
    keyed = [((t + 0.5) / len(l), k, p) for k, l in enumerate(lists) for t, p in enumerate(l)]
    return [p for _, _, p in sorted(keyed)]


def _group_pieces(owner, u, ra, g):
    m = max(1, min(PR // 8, round(g * PR / TGT)))
    return [(owner, u, ra, g, o, n) for o, n in _spread(PR, m)]


def _winddown():
    rem = {(j, r) for j in range(USTAR + 1, NSTEP) for r in range(NS) if j - r > USTAR}
    last_free = I0 - 1
    tot = sum(1 for j, _ in rem if j <= last_free)
    budget = {s: tot * (s - USTAR) / (last_free - USTAR) for s in range(USTAR + 1, last_free + 1)}
    cum = 0
    pieces, ends, owned = [], {}, {}
    for s in range(USTAR + 1, NSTEP):
        groups = {r: 1 for j, r in sorted(rem) if j == s}
        rem -= {(s, r) for r in groups}
        cum += len(groups)

        def fits(cand):
            for s2 in range(s, cand[-1][0]):
                need = sum(1 for c in rem if s < c[0] <= s2 and c not in cand)
                if cum + len(cand) + need > budget[s2] + 1e-9:
                    return False
            return True

        grown = s < last_free
        while grown:
            grown = False
            for r in sorted(groups, key=lambda r: (groups[r], r)):
                g = groups[r]
                cand = [(s + g + e, r + g + e) for e in range(2 if g == 6 else 1)]
                if all(c in rem and c[0] <= last_free for c in cand) and fits(cand):
                    rem -= set(cand)
                    cum += len(cand)
                    groups[r] += len(cand)
                    grown = True
                    break

        done = set()
        for r in sorted(groups):
            if r in done:
                continue
            mate = r + NS // 2
            both = [r]
            if mate in groups and max(groups[r], groups[mate]) <= 2 and _late(s, r) == _late(s, mate):
                both.append(mate)
            done.update(both)
            pieces += _merge([_group_pieces(s, s - q, q, groups[q]) for q in both])
        ends[s] = len(pieces)
        owned[s] = [(s - r, r, g) for r, g in sorted(groups.items())]
    assert not rem

    e0, e1 = ends[I0], ends[I1]
    by_pos = lambda ps: sorted(ps, key=lambda p: (p[2], p[4]))
    k2, v1 = by_pos(pieces[e1:]), by_pos(pieces[e0:e1])
    tag = lambda a, pr, ps: [(a, pr, p) for p in ps]
    los = tag("v", LO, pieces[:e0]) + tag("k", LO, k2[:KLO]) + tag("v", LO, v1[:-VHI]) + tag("v", LO, pieces[e1:])
    his = tag("k", HI, pieces[:e1]) + tag("k", HI, k2[KLO:]) + tag("v", HI, v1[-VHI:])
    plan, lpos, hpos = {}, 0, 0
    for s in range(W0, I0 + 1):
        end = ends[s] if s > USTAR else (s - USTAR) * NP
        lnxt = len(los) if s == I0 else min(len(los), end + AH)
        hnxt = lnxt + (len(his) - len(los) if s >= ADVS else 0)
        plan[s] = _merge([los[lpos:lnxt], his[hpos:hnxt]])
        lpos, hpos = lnxt, hnxt
        assert s < USTAR or hnxt >= ends[s + 1]
        for _, _, (owner, u, ra, g, _, _) in plan[s]:
            assert u + ra + g - 1 - DEPTH < s - 1 and owner - DEPTH < s - 1
    assert lpos == len(los) and hpos == len(his)
    return plan, owned


PIECES = _spread(PR, NP)
WD_PLAN, WD_OWNED = _winddown()
HEAD_GROUPS = {u: ([(u, -u, 4), (u, 4 - u, 3)] if NS + u == 7 else [(u, -u, NS + u)]) for u in range(1 - NS, 0)}


def _owned(j, late=None):
    groups = WD_OWNED[j] if j > USTAR else [(j, 0, NS)]
    return [grp for grp in groups if late is None or _late(j, grp[1]) == late]


def _burst(u, lo, hi):
    return [(u, u, 0, NS, o, n) for o, n in PIECES[lo:hi]]


def _kernel(x_hbm, k_hbm, v_hbm, wq_hbm, wot_hbm, o_hbm,
            kbuf, vbuf, xbuf, wqbuf, wobuf, sbuf, mbuf, qbuf, qall, acc_ref, obuf, p0buf, p1buf, sem):
    K = (k_hbm, kbuf, KS)
    V = (v_hbm, vbuf, VS)

    def sem_of(s0, owner, ra):
        if s0 == VS and isinstance(owner, int) and _late(owner, ra):
            return sem.at[VL0 if owner == I0 else VL2]
        return sem.at[s0 + owner % DEPTH]

    def kv_copy(hbm, buf, s0, owner, u, ra, g, o, n):
        row = ((u + (PK if s0 == KS else 0)) % NS) * PR + o
        if not isinstance(u, int):
            row = pl.multiple_of(row, 8)
        return pltpu.make_async_copy(hbm.at[pl.ds(u + ra, g), pl.ds(row, n)],
                                     buf.at[u % DEPTH, pl.ds(ra, g), pl.ds(o, n)], sem_of(s0, owner, ra))

    def start_pairs(vs, ks):
        for t in range(max(len(vs), len(ks))):
            if t < len(vs):
                kv_copy(*V, *vs[t]).start(priority=LO)
            if t < len(ks):
                kv_copy(*K, *ks[t]).start(priority=HI)

    def start_plan(s):
        for arr, prio, p in WD_PLAN[s]:
            kv_copy(*(K if arr == "k" else V), *p).start(priority=prio)

    def wait_groups(hbm, buf, s0, owner, groups):
        for u, ra, g in groups:
            dst = buf.at[u % DEPTH, pl.ds(ra, g)]
            pltpu.make_async_copy(dst, dst, sem_of(s0, owner, ra)).wait()

    def w_copy(hbm, buf, si, r, o, n):
        return pltpu.make_async_copy(hbm.at[:, pl.ds(r, 8), pl.ds(o, n)],
                                     buf.at[:, pl.ds(r, 8), pl.ds(o, n)], sem.at[si])

    def o_copy(b0, n, si):
        return pltpu.make_async_copy(obuf.at[pl.ds(b0, n)], o_hbm.at[pl.ds(b0, n)], sem.at[si])

    def w_head(buf, i):
        off = (i % H) * DH
        if not isinstance(i, int):
            off = pl.multiple_of(off, DH)
        return buf[:, :, pl.ds(off, DH)].reshape(D, DH)

    def qproj(i):
        b = i // H
        row = (b % (B // XG)) * SQ
        if not isinstance(i, int):
            row = pl.multiple_of(row, 16)
        q = jnp.dot(xbuf[b // (B // XG), pl.ds(row, SQ), :], w_head(wqbuf, i), preferred_element_type=F32)
        return (q * (DH ** -0.5 * LOG2E)).astype(BF)

    def cols(c):
        return slice(c * T, (c + 1) * T)

    def kv_tile(buf, shift, j, c):
        r = (c // TP + shift) % NS
        return buf[(j + DEPTH - r) % DEPTH, r, pl.ds((c % TP) * T, T), :]

    def qk_tile(st, q, j, c):
        s = jax.lax.dot_general(q, kv_tile(kbuf, PK, j, c), NT_DIMS, preferred_element_type=F32)
        sbuf[:, cols(c)] = s
        st["mx"] = s if c == 0 else jnp.maximum(st["mx"], s)

    def row_max(st):
        return jnp.broadcast_to(jnp.max(st["mx"], axis=-1, keepdims=True), (SQ, T))

    def exp_tile(st, m, c):
        p = jnp.exp2(sbuf[:, cols(c)] - m)
        st["l"] = p if c == 0 else st["l"] + p
        return p.astype(BF)

    def inv_sum(st):
        return pl.reciprocal(jnp.sum(st["l"], axis=-1, keepdims=True), approx=False)

    def pv_tile(st, p, j, c):
        pv = jnp.dot(p, kv_tile(vbuf, 0, j, c), preferred_element_type=F32)
        st["o"] = pv if c == 0 else st["o"] + pv

    def oproj(st, rinv, j):
        o = (st["o"] * rinv).astype(BF)
        return jax.lax.dot_general(o, w_head(wobuf, j), NT_DIMS, preferred_element_type=F32)

    for o, n in _spread(XR, XP):
        pltpu.make_async_copy(x_hbm.at[:, pl.ds(o, n)], xbuf.at[:, pl.ds(o, n)], sem.at[XS]).start(priority=LO)
    for r in range(0, WR, 8):
        for o, n in _spread(H * DH, WC, 128):
            w_copy(wot_hbm, wobuf, WOS, r, o, n).start(priority=LO)
            w_copy(wq_hbm, wqbuf, WQS, r, o, n).start(priority=HI)
    head = []
    for u, groups in HEAD_GROUPS.items():
        head += _merge([_group_pieces(u, *grp) for grp in groups])
    start_pairs(head[:Q1], head[:Q1])
    pltpu.make_async_copy(x_hbm, xbuf, sem.at[XS]).wait()
    pltpu.make_async_copy(wq_hbm, wqbuf, sem.at[WQS]).wait()

    def q_early(j, carry):
        qall[j - (W0 + 1)] = qproj(j)
        return carry

    pos = Q1
    for o, n in _spread(NQ - 1, QCH, 1):
        jax.lax.fori_loop(W0 + 2 + o, W0 + 2 + o + n, q_early, 0)
        start_pairs(head[pos:pos + QG], head[pos:pos + QG])
        pos += QG
    start_pairs(head[pos:], head[pos:])
    ks = _burst(0, 0, NP) + _burst(1, 0, NP) + _burst(2, 0, PK0)
    start_pairs([], ks[:PK0 - PV0])
    start_pairs(_burst(0, 0, NP) + _burst(1, 0, NP) + _burst(2, 0, PV0), ks[PK0 - PV0:])
    acc_ref[...] = jnp.zeros_like(acc_ref)

    pltpu.make_async_copy(wot_hbm, wobuf, sem.at[WOS]).wait()
    for u, groups in HEAD_GROUPS.items():
        wait_groups(*K, u, groups)
    wait_groups(*K, 0, _owned(0))
    st0 = {}
    q0 = qproj(0)
    qbuf[...] = qproj(1)
    for c in range(NT):
        qk_tile(st0, q0, 0, c)
    mbuf[...] = row_max(st0)

    def compute(i, q, with_q):
        st = {}
        m = mbuf[...]
        for c in range(NT + SKEW):
            if c < NT:
                pv_tile(st, exp_tile(st, m, c), i, c)
            if c == 0 and with_q:
                q_next = qproj(i + 2)
            if c >= SKEW:
                qk_tile(st, q, i + 1, c - SKEW)
        acc_ref[...] += oproj(st, inv_sum(st), i)
        if with_q:
            qbuf[...] = q_next
        mbuf[...] = row_max(st)

        @pl.when(i % H == H - 1)
        def _():
            obuf[i // H] = acc_ref[...].astype(BF)
            acc_ref[...] = jnp.zeros_like(acc_ref)

    def steady_step(i, carry):
        start_pairs(_burst(i + 2, PV0, NP) + _burst(i + 3, 0, PV0),
                    _burst(i + 2, PK0, NP) + _burst(i + 3, 0, PK0))

        @pl.when(i == 0)
        def _():
            for u, groups in HEAD_GROUPS.items():
                wait_groups(*V, u, groups)

        wait_groups(*K, i + 1, [(i + 1, 0, NS)])
        wait_groups(*V, i, [(i, 0, NS)])
        compute(i, qbuf[...], True)
        return carry

    jax.lax.fori_loop(0, W0, steady_step, 0)
    qall[0] = qbuf[...]

    def winddown_step(i, carry):
        def dispatch(lo, hi):
            if hi - lo > 1:
                mid = (lo + hi) // 2
                jax.lax.cond(i < mid, lambda: dispatch(lo, mid), lambda: dispatch(mid, hi))
                return
            if lo == W0:
                start_pairs(_burst(USTAR, PV0, NP), _burst(USTAR, PK0, NP))
            start_plan(lo)
            wait_groups(*K, lo + 1, _owned(lo + 1))
            wait_groups(*V, lo, _owned(lo))

        dispatch(W0, I0)
        compute(i, qall[i - W0], False)
        return carry

    jax.lax.fori_loop(W0, I0, winddown_step, 0)

    s0, s1, s2 = {}, {}, {}
    start_plan(I0)
    wait_groups(*K, I1, _owned(I1))
    wait_groups(*V, I0, _owned(I0, late=False))
    m0 = mbuf[...]
    q = qall[NQ - 2]
    for c in range(NT):
        p = exp_tile(s0, m0, c)
        if c < TA:
            pv_tile(s0, p, I0, c)
        else:
            p0buf[:, cols(c - TA)] = p
        qk_tile(s1, q, I1, c)
    r0 = inv_sum(s0)
    m1 = row_max(s1)
    wait_groups(*V, I0, _owned(I0, late=True))
    wait_groups(*K, I2, _owned(I2))
    q = qall[NQ - 1]
    for c in range(TA, NT):
        pv_tile(s0, p0buf[:, cols(c - TA)], I0, c)
    for c in range(NT):
        p1buf[:, cols(c)] = exp_tile(s1, m1, c)
        qk_tile(s2, q, I2, c)
    acc_ref[...] += oproj(s0, r0, I0)
    r1 = inv_sum(s1)
    m2 = row_max(s2)
    wait_groups(*V, I1, _owned(I1))
    for c in range(NT):
        pv_tile(s1, p1buf[:, cols(c)], I1, c)
    acc_ref[...] += oproj(s1, r1, I1)
    wait_groups(*V, I2, _owned(I2, late=False))
    o_copy(0, B - 1, OS0).start(priority=LO)
    wait_groups(*V, I2, _owned(I2, late=True))
    for c in range(NT):
        pv_tile(s2, exp_tile(s2, m2, c), I2, c)
    obuf[B - 1] = (acc_ref[...] + oproj(s2, inv_sum(s2), I2)).astype(BF)
    o_copy(B - 1, 1, OS1).start(priority=HI)
    o_copy(0, B - 1, OS0).wait()
    o_copy(B - 1, 1, OS1).wait()


@jax.jit
def pallas_standalone__mha_block_cached__near_ridge_kernel(
    x: jax.Array,
    k_cache: jax.Array,
    v_cache: jax.Array,
    wq: jax.Array,
    wo: jax.Array,
):
    any_spec = pl.BlockSpec(memory_space=pl.ANY)
    return pl.pallas_call(
        _kernel,
        in_specs=[any_spec] * 5,
        out_specs=any_spec,
        out_shape=jax.ShapeDtypeStruct((B, SQ, D), x.dtype),
        scratch_shapes=[
            pltpu.VMEM((DEPTH, NS, PR, DH), BF),
            pltpu.VMEM((DEPTH, NS, PR, DH), BF),
            pltpu.VMEM((XG, XR, D), BF),
            pltpu.VMEM((WG, WR, H * DH), BF),
            pltpu.VMEM((WG, WR, H * DH), BF),
            pltpu.VMEM((SQ, SK), F32),
            pltpu.VMEM((SQ, T), F32),
            pltpu.VMEM((SQ, DH), BF),
            pltpu.VMEM((NQ, SQ, DH), BF),
            pltpu.VMEM((SQ, D), F32),
            pltpu.VMEM((B, SQ, D), BF),
            pltpu.VMEM((SQ, (NT - TA) * T), BF),
            pltpu.VMEM((SQ, SK), BF),
            pltpu.SemaphoreType.DMA((NSEM,)),
        ],
        compiler_params=pltpu.CompilerParams(
            vmem_limit_bytes=64 * 1024 * 1024,
            disable_bounds_checks=True,
            disable_semaphore_checks=True,
        ),
    )(
        x.reshape(XG, XR, D),
        k_cache.reshape(NSTEP, SK, DH),
        v_cache.reshape(NSTEP, SK, DH),
        wq.reshape(WG, WR, H * DH),
        wo.T.reshape(WG, WR, H * DH),
    )
```

```python
import jax
import jax.numpy as jnp
import jax.experimental.pallas as pl
import jax.experimental.pallas.tpu as pltpu

B, SQ, D = 8, 144, 448
H, SK, DH = 16, 2048, 256
NSTEP = B * H

T = 128
NT = SK // T
SKEW = 2

NS = 8
PR = SK // NS
TP = NT // NS
DEPTH = 16
NP = 26
PV0, PK0 = 3, 4
PK = NS - 1
USTAR = 110
W0 = USTAR - 2
NQ = NSTEP - 1 - W0
AH = 54
TGT = 88
I0, I1, I2 = NSTEP - 3, NSTEP - 2, NSTEP - 1
TA = 12
KLO, VHI = 9, 11
LATE2 = (3, 6, 7)
ADVS = 122

WG, WC = 4, 6
WR = D // WG
XG, XP = 2, 26
XR = B * SQ // XG
QCH, Q1, QG = 3, 28, 20

HI, LO = 0, 1
NT_DIMS = (((1,), (1,)), ((), ()))
BF = jnp.bfloat16
F32 = jnp.float32

KS, VS = 0, DEPTH
WQS, WOS, XS, OS0, OS1, VL0, VL2 = range(2 * DEPTH, 2 * DEPTH + 7)
NSEM = VL2 + 1


def _late(j, r):
    return (j == I0 and r * TP >= TA) or (j == I2 and r in LATE2)


def _spread(total, m, g=8):
    units = total // g
    out, o = [], 0
    for j in range(m):
        e = ((j + 1) * units) // m * g
        out.append((o, e - o))
        o = e
    return out


def _merge(lists):
    keyed = [((t + 0.5) / len(l), k, p) for k, l in enumerate(lists) for t, p in enumerate(l)]
    return [p for _, _, p in sorted(keyed)]


def _group_pieces(owner, u, ra, g):
    m = max(1, min(PR // 8, round(g * PR / TGT)))
    return [(owner, u, ra, g, o, n) for o, n in _spread(PR, m)]


def _winddown():
    rem = {(j, r) for j in range(USTAR + 1, NSTEP) for r in range(NS) if j - r > USTAR}
    last_free = I0 - 1
    tot = sum(1 for j, _ in rem if j <= last_free)
    budget = {s: tot * (s - USTAR) / (last_free - USTAR) for s in range(USTAR + 1, last_free + 1)}
    cum = 0
    pieces, ends, owned = [], {}, {}
    for s in range(USTAR + 1, NSTEP):
        groups = {r: 1 for j, r in sorted(rem) if j == s}
        rem -= {(s, r) for r in groups}
        cum += len(groups)

        def fits(cand):
            for s2 in range(s, cand[-1][0]):
                need = sum(1 for c in rem if s < c[0] <= s2 and c not in cand)
                if cum + len(cand) + need > budget[s2] + 1e-9:
                    return False
            return True

        grown = s < last_free
        while grown:
            grown = False
            for r in sorted(groups, key=lambda r: (groups[r], r)):
                g = groups[r]
                cand = [(s + g + e, r + g + e) for e in range(2 if g == 6 else 1)]
                if all(c in rem and c[0] <= last_free for c in cand) and fits(cand):
                    rem -= set(cand)
                    cum += len(cand)
                    groups[r] += len(cand)
                    grown = True
                    break

        done = set()
        for r in sorted(groups):
            if r in done:
                continue
            mate = r + NS // 2
            both = [r]
            if mate in groups and max(groups[r], groups[mate]) <= 2 and _late(s, r) == _late(s, mate):
                both.append(mate)
            done.update(both)
            pieces += _merge([_group_pieces(s, s - q, q, groups[q]) for q in both])
        ends[s] = len(pieces)
        owned[s] = [(s - r, r, g) for r, g in sorted(groups.items())]
    assert not rem

    e0, e1 = ends[I0], ends[I1]
    by_pos = lambda ps: sorted(ps, key=lambda p: (p[2], p[4]))
    k2, v1 = by_pos(pieces[e1:]), by_pos(pieces[e0:e1])
    tag = lambda a, pr, ps: [(a, pr, p) for p in ps]
    los = tag("v", LO, pieces[:e0]) + tag("k", LO, k2[:KLO]) + tag("v", LO, v1[:-VHI]) + tag("v", LO, pieces[e1:])
    his = tag("k", HI, pieces[:e1]) + tag("k", HI, k2[KLO:]) + tag("v", HI, v1[-VHI:])
    plan, lpos, hpos = {}, 0, 0
    for s in range(W0, I0 + 1):
        end = ends[s] if s > USTAR else (s - USTAR) * NP
        lnxt = len(los) if s == I0 else min(len(los), end + AH)
        hnxt = lnxt + (len(his) - len(los) if s >= ADVS else 0)
        plan[s] = _merge([los[lpos:lnxt], his[hpos:hnxt]])
        lpos, hpos = lnxt, hnxt
        assert s < USTAR or hnxt >= ends[s + 1]
        for _, _, (owner, u, ra, g, _, _) in plan[s]:
            assert u + ra + g - 1 - DEPTH < s - 1 and owner - DEPTH < s - 1
    assert lpos == len(los) and hpos == len(his)
    return plan, owned


PIECES = _spread(PR, NP)
WD_PLAN, WD_OWNED = _winddown()
HEAD_GROUPS = {u: ([(u, -u, 4), (u, 4 - u, 3)] if NS + u == 7 else [(u, -u, NS + u)]) for u in range(1 - NS, 0)}


def _owned(j, late=None):
    groups = WD_OWNED[j] if j > USTAR else [(j, 0, NS)]
    return [grp for grp in groups if late is None or _late(j, grp[1]) == late]


def _burst(u, lo, hi):
    return [(u, u, 0, NS, o, n) for o, n in PIECES[lo:hi]]


def _kernel(x_hbm, k_hbm, v_hbm, wq_hbm, wot_hbm, o_hbm,
            kbuf, vbuf, xbuf, wqbuf, wobuf, sbuf, mbuf, qbuf, qall, acc_ref, obuf, p0buf, p1buf, sem):
    K = (k_hbm, kbuf, KS)
    V = (v_hbm, vbuf, VS)

    def sem_of(s0, owner, ra):
        if s0 == VS and isinstance(owner, int) and _late(owner, ra):
            return sem.at[VL0 if owner == I0 else VL2]
        return sem.at[s0 + owner % DEPTH]

    def kv_copy(hbm, buf, s0, owner, u, ra, g, o, n):
        row = ((u + (PK if s0 == KS else 0)) % NS) * PR + o
        if not isinstance(u, int):
            row = pl.multiple_of(row, 8)
        return pltpu.make_async_copy(hbm.at[pl.ds(u + ra, g), pl.ds(row, n)],
                                     buf.at[u % DEPTH, pl.ds(ra, g), pl.ds(o, n)], sem_of(s0, owner, ra))

    def start_pairs(vs, ks):
        for t in range(max(len(vs), len(ks))):
            if t < len(vs):
                kv_copy(*V, *vs[t]).start(priority=LO)
            if t < len(ks):
                kv_copy(*K, *ks[t]).start(priority=HI)

    def start_plan(s):
        for arr, prio, p in WD_PLAN[s]:
            kv_copy(*(K if arr == "k" else V), *p).start(priority=prio)

    def wait_groups(hbm, buf, s0, owner, groups):
        for u, ra, g in groups:
            dst = buf.at[u % DEPTH, pl.ds(ra, g)]
            pltpu.make_async_copy(dst, dst, sem_of(s0, owner, ra)).wait()

    def w_copy(hbm, buf, si, r, o, n):
        return pltpu.make_async_copy(hbm.at[:, pl.ds(r, 8), pl.ds(o, n)],
                                     buf.at[:, pl.ds(r, 8), pl.ds(o, n)], sem.at[si])

    def o_copy(b0, n, si):
        return pltpu.make_async_copy(obuf.at[pl.ds(b0, n)], o_hbm.at[pl.ds(b0, n)], sem.at[si])

    def w_head(buf, i):
        off = (i % H) * DH
        if not isinstance(i, int):
            off = pl.multiple_of(off, DH)
        return buf[:, :, pl.ds(off, DH)].reshape(D, DH)

    def qproj(i):
        b = i // H
        row = (b % (B // XG)) * SQ
        if not isinstance(i, int):
            row = pl.multiple_of(row, 16)
        q = jnp.dot(xbuf[b // (B // XG), pl.ds(row, SQ), :], w_head(wqbuf, i), preferred_element_type=F32)
        return (q * DH ** -0.5).astype(BF)

    def cols(c):
        return slice(c * T, (c + 1) * T)

    def kv_tile(buf, shift, j, c):
        r = (c // TP + shift) % NS
        return buf[(j + DEPTH - r) % DEPTH, r, pl.ds((c % TP) * T, T), :]

    def qk_tile(st, q, j, c):
        s = jax.lax.dot_general(q, kv_tile(kbuf, PK, j, c), NT_DIMS, preferred_element_type=F32)
        sbuf[:, cols(c)] = s.astype(BF).astype(F32)
        st["mx"] = jnp.maximum(st["mx"], s) if "mx" in st else s

    def row_max(st):
        return jnp.broadcast_to(jnp.max(st["mx"].astype(BF).astype(F32), axis=-1, keepdims=True), (SQ, T))

    def exp_tile(st, m, c):
        p = jnp.exp(sbuf[:, cols(c)] - m)
        st["l"] = st["l"] + p if "l" in st else p
        return p.astype(BF)

    def inv_sum(st):
        return 1.0 / jnp.sum(st["l"], axis=-1, keepdims=True)

    def pv_tile(st, p, j, c):
        pv = jnp.dot(p, kv_tile(vbuf, 0, j, c), preferred_element_type=F32)
        st["o"] = st["o"] + pv if "o" in st else pv

    def onorm(st, rinv):
        return (st["o"] * rinv).astype(BF)

    def oproj(o, j):
        return jax.lax.dot_general(o, w_head(wobuf, j), NT_DIMS, preferred_element_type=F32)

    for o, n in _spread(XR, XP):
        pltpu.make_async_copy(x_hbm.at[:, pl.ds(o, n)], xbuf.at[:, pl.ds(o, n)], sem.at[XS]).start(priority=LO)
    for r in range(0, WR, 8):
        for o, n in _spread(H * DH, WC, 128):
            w_copy(wot_hbm, wobuf, WOS, r, o, n).start(priority=LO)
            w_copy(wq_hbm, wqbuf, WQS, r, o, n).start(priority=HI)
    head = []
    for u, groups in HEAD_GROUPS.items():
        head += _merge([_group_pieces(u, *grp) for grp in groups])
    start_pairs(head[:Q1], head[:Q1])
    pltpu.make_async_copy(x_hbm, xbuf, sem.at[XS]).wait()
    pltpu.make_async_copy(wq_hbm, wqbuf, sem.at[WQS]).wait()

    def q_early(j, carry):
        qall[j - (W0 + 1)] = qproj(j)
        return carry

    pos = Q1
    for o, n in _spread(NQ - 1, QCH, 1):
        jax.lax.fori_loop(W0 + 2 + o, W0 + 2 + o + n, q_early, 0)
        start_pairs(head[pos:pos + QG], head[pos:pos + QG])
        pos += QG
    start_pairs(head[pos:], head[pos:])
    ks = _burst(0, 0, NP) + _burst(1, 0, NP) + _burst(2, 0, PK0)
    start_pairs([], ks[:PK0 - PV0])
    start_pairs(_burst(0, 0, NP) + _burst(1, 0, NP) + _burst(2, 0, PV0), ks[PK0 - PV0:])
    acc_ref[...] = jnp.zeros_like(acc_ref)

    pltpu.make_async_copy(wot_hbm, wobuf, sem.at[WOS]).wait()
    for u, groups in HEAD_GROUPS.items():
        wait_groups(*K, u, groups)
    wait_groups(*K, 0, _owned(0))
    st0 = {}
    q0 = qproj(0)
    qbuf[...] = qproj(1)
    for c in range(NT):
        qk_tile(st0, q0, 0, c)
    mbuf[...] = row_max(st0)

    def compute(i, q, with_q):
        st = {}
        m = mbuf[...]
        for c in range(NT + SKEW):
            if c < NT:
                pv_tile(st, exp_tile(st, m, c), i, c)
            if c == 0 and with_q:
                q_next = qproj(i + 2)
            if c >= SKEW:
                qk_tile(st, q, i + 1, c - SKEW)
        acc_ref[...] += oproj(onorm(st, inv_sum(st)), i)
        if with_q:
            qbuf[...] = q_next
        mbuf[...] = row_max(st)

        @pl.when(i % H == H - 1)
        def _():
            obuf[i // H] = acc_ref[...].astype(BF)
            acc_ref[...] = jnp.zeros_like(acc_ref)

    def steady_step(i, carry):
        start_pairs(_burst(i + 2, PV0, NP) + _burst(i + 3, 0, PV0),
                    _burst(i + 2, PK0, NP) + _burst(i + 3, 0, PK0))

        @pl.when(i == 0)
        def _():
            for u, groups in HEAD_GROUPS.items():
                wait_groups(*V, u, groups)

        wait_groups(*K, i + 1, [(i + 1, 0, NS)])
        wait_groups(*V, i, [(i, 0, NS)])
        compute(i, qbuf[...], True)
        return carry

    jax.lax.fori_loop(0, W0, steady_step, 0)
    qall[0] = qbuf[...]

    def winddown_step(i, carry):
        def dispatch(lo, hi):
            if hi - lo > 1:
                mid = (lo + hi) // 2
                jax.lax.cond(i < mid, lambda: dispatch(lo, mid), lambda: dispatch(mid, hi))
                return
            if lo == W0:
                start_pairs(_burst(USTAR, PV0, NP), _burst(USTAR, PK0, NP))
            start_plan(lo)
            wait_groups(*K, lo + 1, _owned(lo + 1))
            wait_groups(*V, lo, _owned(lo))

        dispatch(W0, I0)
        compute(i, qall[i - W0], False)
        return carry

    jax.lax.fori_loop(W0, I0, winddown_step, 0)

    s0, s1, s2 = {}, {}, {}
    start_plan(I0)
    wait_groups(*K, I1, _owned(I1))
    wait_groups(*V, I0, _owned(I0, late=False))
    m0 = mbuf[...]
    q = qall[NQ - 2]
    for c in range(NT):
        p = exp_tile(s0, m0, c)
        if c < TA:
            pv_tile(s0, p, I0, c)
        else:
            p0buf[:, cols(c - TA)] = p
        qk_tile(s1, q, I1, c)
    r0 = inv_sum(s0)
    m1 = row_max(s1)
    wait_groups(*V, I0, _owned(I0, late=True))
    wait_groups(*K, I2, _owned(I2))
    q = qall[NQ - 1]
    for c in range(TA, NT):
        pv_tile(s0, p0buf[:, cols(c - TA)], I0, c)
    for c in range(NT):
        p1buf[:, cols(c)] = exp_tile(s1, m1, c)
        qk_tile(s2, q, I2, c)
    acc_ref[...] += oproj(onorm(s0, r0), I0)
    r1 = inv_sum(s1)
    m2 = row_max(s2)
    wait_groups(*V, I1, _owned(I1))
    for c in range(NT):
        pv_tile(s1, p1buf[:, cols(c)], I1, c)
    o1 = onorm(s1, r1)
    wait_groups(*V, I2, _owned(I2, late=False))
    o_copy(0, B - 1, OS0).start(priority=LO)
    early = [c for c in range(NT) if not _late(I2, c // TP)]
    acc_ref[...] += oproj(o1, I1)
    for c in early:
        pv_tile(s2, exp_tile(s2, m2, c), I2, c)
    wait_groups(*V, I2, _owned(I2, late=True))
    for c in range(NT):
        if c not in early:
            pv_tile(s2, exp_tile(s2, m2, c), I2, c)
    obuf[B - 1] = (acc_ref[...] + oproj(onorm(s2, inv_sum(s2)), I2)).astype(BF)
    o_copy(B - 1, 1, OS1).start(priority=HI)
    o_copy(0, B - 1, OS0).wait()
    o_copy(B - 1, 1, OS1).wait()


@jax.jit
def pallas_standalone__mha_block_cached__near_ridge_kernel(
    x: jax.Array,
    k_cache: jax.Array,
    v_cache: jax.Array,
    wq: jax.Array,
    wo: jax.Array,
):
    any_spec = pl.BlockSpec(memory_space=pl.ANY)
    return pl.pallas_call(
        _kernel,
        in_specs=[any_spec] * 5,
        out_specs=any_spec,
        out_shape=jax.ShapeDtypeStruct((B, SQ, D), x.dtype),
        scratch_shapes=[
            pltpu.VMEM((DEPTH, NS, PR, DH), BF),
            pltpu.VMEM((DEPTH, NS, PR, DH), BF),
            pltpu.VMEM((XG, XR, D), BF),
            pltpu.VMEM((WG, WR, H * DH), BF),
            pltpu.VMEM((WG, WR, H * DH), BF),
            pltpu.VMEM((SQ, SK), F32),
            pltpu.VMEM((SQ, T), F32),
            pltpu.VMEM((SQ, DH), BF),
            pltpu.VMEM((NQ, SQ, DH), BF),
            pltpu.VMEM((SQ, D), F32),
            pltpu.VMEM((B, SQ, D), BF),
            pltpu.VMEM((SQ, (NT - TA) * T), BF),
            pltpu.VMEM((SQ, SK), BF),
            pltpu.SemaphoreType.DMA((NSEM,)),
        ],
        compiler_params=pltpu.CompilerParams(
            vmem_limit_bytes=64 * 1024 * 1024,
            disable_bounds_checks=True,
            disable_semaphore_checks=True,
        ),
    )(
        x.reshape(XG, XR, D),
        k_cache.reshape(NSTEP, SK, DH),
        v_cache.reshape(NSTEP, SK, DH),
        wq.reshape(WG, WR, H * DH),
        wo.T.reshape(WG, WR, H * DH),
    )
```

```python
import jax
import jax.numpy as jnp
import jax.experimental.pallas as pl
import jax.experimental.pallas.tpu as pltpu

B, SQ, D = 8, 144, 448
H, SK, DH = 16, 2048, 256
NSTEP = B * H

T = 128
NT = SK // T
SKEW = 2

NS = 8
PR = SK // NS
TP = NT // NS
DEPTH = 16
NP = 26
PV0, PK0 = 3, 4
PK = NS - 1
USTAR = 110
W0 = USTAR - 2
NQ = NSTEP - 1 - W0
AH = 54
TGT = 88
I0, I1, I2 = NSTEP - 3, NSTEP - 2, NSTEP - 1
TA = 12
KLO, VHI = 9, 11
LATE2 = (3, 6, 7)
ADVS = 122

WG, WC = 4, 6
WR = D // WG
XG, XP = 2, 26
XR = B * SQ // XG
QCH, Q1, QG = 3, 28, 20

HI, LO = 0, 1
NT_DIMS = (((1,), (1,)), ((), ()))
BF = jnp.bfloat16
F32 = jnp.float32

KS, VS = 0, DEPTH
WQS, WOS, XS, OS0, OS1, VL0, VL2 = range(2 * DEPTH, 2 * DEPTH + 7)
NSEM = VL2 + 1


def _late(j, r):
    return (j == I0 and r * TP >= TA) or (j == I2 and r in LATE2)


def _spread(total, m, g=8):
    units = total // g
    out, o = [], 0
    for j in range(m):
        e = ((j + 1) * units) // m * g
        out.append((o, e - o))
        o = e
    return out


def _merge(lists):
    keyed = [((t + 0.5) / len(l), k, p) for k, l in enumerate(lists) for t, p in enumerate(l)]
    return [p for _, _, p in sorted(keyed)]


def _group_pieces(owner, u, ra, g):
    m = max(1, min(PR // 8, round(g * PR / TGT)))
    return [(owner, u, ra, g, o, n) for o, n in _spread(PR, m)]


def _winddown():
    rem = {(j, r) for j in range(USTAR + 1, NSTEP) for r in range(NS) if j - r > USTAR}
    last_free = I0 - 1
    tot = sum(1 for j, _ in rem if j <= last_free)
    budget = {s: tot * (s - USTAR) / (last_free - USTAR) for s in range(USTAR + 1, last_free + 1)}
    cum = 0
    pieces, ends, owned = [], {}, {}
    for s in range(USTAR + 1, NSTEP):
        groups = {r: 1 for j, r in sorted(rem) if j == s}
        rem -= {(s, r) for r in groups}
        cum += len(groups)

        def fits(cand):
            for s2 in range(s, cand[-1][0]):
                need = sum(1 for c in rem if s < c[0] <= s2 and c not in cand)
                if cum + len(cand) + need > budget[s2] + 1e-9:
                    return False
            return True

        grown = s < last_free
        while grown:
            grown = False
            for r in sorted(groups, key=lambda r: (groups[r], r)):
                g = groups[r]
                cand = [(s + g + e, r + g + e) for e in range(2 if g == 6 else 1)]
                if all(c in rem and c[0] <= last_free for c in cand) and fits(cand):
                    rem -= set(cand)
                    cum += len(cand)
                    groups[r] += len(cand)
                    grown = True
                    break

        done = set()
        for r in sorted(groups):
            if r in done:
                continue
            mate = r + NS // 2
            both = [r]
            if mate in groups and max(groups[r], groups[mate]) <= 2 and _late(s, r) == _late(s, mate):
                both.append(mate)
            done.update(both)
            pieces += _merge([_group_pieces(s, s - q, q, groups[q]) for q in both])
        ends[s] = len(pieces)
        owned[s] = [(s - r, r, g) for r, g in sorted(groups.items())]
    assert not rem

    e0, e1 = ends[I0], ends[I1]
    by_pos = lambda ps: sorted(ps, key=lambda p: (p[2], p[4]))
    k2, v1 = by_pos(pieces[e1:]), by_pos(pieces[e0:e1])
    tag = lambda a, pr, ps: [(a, pr, p) for p in ps]
    los = tag("v", LO, pieces[:e0]) + tag("k", LO, k2[:KLO]) + tag("v", LO, v1[:-VHI]) + tag("v", LO, pieces[e1:])
    his = tag("k", HI, pieces[:e1]) + tag("k", HI, k2[KLO:]) + tag("v", HI, v1[-VHI:])
    plan, lpos, hpos = {}, 0, 0
    for s in range(W0, I0 + 1):
        end = ends[s] if s > USTAR else (s - USTAR) * NP
        lnxt = len(los) if s == I0 else min(len(los), end + AH)
        hnxt = lnxt + (len(his) - len(los) if s >= ADVS else 0)
        plan[s] = _merge([los[lpos:lnxt], his[hpos:hnxt]])
        lpos, hpos = lnxt, hnxt
        assert s < USTAR or hnxt >= ends[s + 1]
        for _, _, (owner, u, ra, g, _, _) in plan[s]:
            assert u + ra + g - 1 - DEPTH < s - 1 and owner - DEPTH < s - 1
    assert lpos == len(los) and hpos == len(his)
    return plan, owned


PIECES = _spread(PR, NP)
WD_PLAN, WD_OWNED = _winddown()
HEAD_GROUPS = {u: ([(u, -u, 4), (u, 4 - u, 3)] if NS + u == 7 else [(u, -u, NS + u)]) for u in range(1 - NS, 0)}


def _burst(u, lo, hi):
    return [(u, u, 0, NS, o, n) for o, n in PIECES[lo:hi]]


def _kernel(x_hbm, k_hbm, v_hbm, wq_hbm, wot_hbm, o_hbm,
            kbuf, vbuf, xbuf, wqbuf, wobuf, sbuf, mbuf, qbuf, qall, acc_ref, obuf, p0buf, p1buf, sem):
    K = (k_hbm, kbuf, KS)
    V = (v_hbm, vbuf, VS)

    def sem_of(s0, owner, ra):
        if s0 == VS and isinstance(owner, int) and _late(owner, ra):
            return sem.at[VL0 if owner == I0 else VL2]
        return sem.at[s0 + owner % DEPTH]

    def kv_copy(hbm, buf, s0, owner, u, ra, g, o, n):
        row = ((u + (PK if s0 == KS else 0)) % NS) * PR + o
        if not isinstance(u, int):
            row = pl.multiple_of(row, 8)
        return pltpu.make_async_copy(hbm.at[pl.ds(u + ra, g), pl.ds(row, n)],
                                     buf.at[u % DEPTH, pl.ds(ra, g), pl.ds(o, n)], sem_of(s0, owner, ra))

    def start_pairs(vs, ks):
        for t in range(max(len(vs), len(ks))):
            if t < len(vs):
                kv_copy(*V, *vs[t]).start(priority=LO)
            if t < len(ks):
                kv_copy(*K, *ks[t]).start(priority=HI)

    def start_plan(s):
        for arr, prio, p in WD_PLAN[s]:
            kv_copy(*(K if arr == "k" else V), *p).start(priority=prio)

    def wait_burst(hbm, buf, s0, u, ra=0):
        dst = buf.at[u % DEPTH, pl.ds(ra, NS - ra)]
        pltpu.make_async_copy(dst, dst, sem.at[s0 + u % DEPTH]).wait()

    def wait_slab(arr, j, late=None):
        if j <= USTAR:
            wait_burst(*arr, j)
            return
        for grp in WD_OWNED[j]:
            if late is None or _late(j, grp[1]) == late:
                for p in _group_pieces(j, *grp):
                    kv_copy(*arr, *p).wait()

    def w_copy(hbm, buf, si, r, o, n):
        return pltpu.make_async_copy(hbm.at[:, pl.ds(r, 8), pl.ds(o, n)],
                                     buf.at[:, pl.ds(r, 8), pl.ds(o, n)], sem.at[si])

    def o_copy(b0, n, si):
        return pltpu.make_async_copy(obuf.at[pl.ds(b0, n)], o_hbm.at[pl.ds(b0, n)], sem.at[si])

    def w_head(buf, i):
        off = (i % H) * DH
        if not isinstance(i, int):
            off = pl.multiple_of(off, DH)
        return buf[:, :, pl.ds(off, DH)].reshape(D, DH)

    def qproj(i):
        b = i // H
        row = (b % (B // XG)) * SQ
        if not isinstance(i, int):
            row = pl.multiple_of(row, 16)
        q = jnp.dot(xbuf[b // (B // XG), pl.ds(row, SQ), :], w_head(wqbuf, i), preferred_element_type=F32)
        return (q * DH ** -0.5).astype(BF)

    def cols(c):
        return slice(c * T, (c + 1) * T)

    def kv_tile(buf, shift, j, c):
        r = (c // TP + shift) % NS
        return buf[(j + DEPTH - r) % DEPTH, r, pl.ds((c % TP) * T, T), :]

    def qk_tile(st, q, j, c):
        s = jax.lax.dot_general(q, kv_tile(kbuf, PK, j, c), NT_DIMS, preferred_element_type=F32)
        sbuf[:, cols(c)] = s.astype(BF).astype(F32)
        st["mx"] = jnp.maximum(st["mx"], s) if "mx" in st else s

    def row_max(st):
        return jnp.broadcast_to(jnp.max(st["mx"].astype(BF).astype(F32), axis=-1, keepdims=True), (SQ, T))

    def exp_tile(st, m, c):
        p = jnp.exp(sbuf[:, cols(c)] - m)
        st["l"] = st["l"] + p if "l" in st else p
        return p.astype(BF)

    def inv_sum(st):
        return 1.0 / jnp.sum(st["l"], axis=-1, keepdims=True)

    def pv_tile(st, p, j, c):
        pv = jnp.dot(p, kv_tile(vbuf, 0, j, c), preferred_element_type=F32)
        st["o"] = st["o"] + pv if "o" in st else pv

    def onorm(st, rinv):
        return (st["o"] * rinv).astype(BF)

    def oproj(o, j):
        return jax.lax.dot_general(o, w_head(wobuf, j), NT_DIMS, preferred_element_type=F32)

    for o, n in _spread(XR, XP):
        pltpu.make_async_copy(x_hbm.at[:, pl.ds(o, n)], xbuf.at[:, pl.ds(o, n)], sem.at[XS]).start(priority=LO)
    for r in range(0, WR, 8):
        for o, n in _spread(H * DH, WC, 128):
            w_copy(wot_hbm, wobuf, WOS, r, o, n).start(priority=LO)
            w_copy(wq_hbm, wqbuf, WQS, r, o, n).start(priority=HI)
    head = []
    for u, groups in HEAD_GROUPS.items():
        head += _merge([_group_pieces(u, *grp) for grp in groups])
    start_pairs(head[:Q1], head[:Q1])
    pltpu.make_async_copy(x_hbm, xbuf, sem.at[XS]).wait()
    pltpu.make_async_copy(wq_hbm, wqbuf, sem.at[WQS]).wait()

    def q_early(j, carry):
        qall[j - (W0 + 1)] = qproj(j)
        return carry

    pos = Q1
    for o, n in _spread(NQ - 1, QCH, 1):
        jax.lax.fori_loop(W0 + 2 + o, W0 + 2 + o + n, q_early, 0)
        start_pairs(head[pos:pos + QG], head[pos:pos + QG])
        pos += QG
    start_pairs(head[pos:], head[pos:])
    ks = _burst(0, 0, NP) + _burst(1, 0, NP) + _burst(2, 0, PK0)
    start_pairs([], ks[:PK0 - PV0])
    start_pairs(_burst(0, 0, NP) + _burst(1, 0, NP) + _burst(2, 0, PV0), ks[PK0 - PV0:])
    acc_ref[...] = jnp.zeros_like(acc_ref)

    pltpu.make_async_copy(wot_hbm, wobuf, sem.at[WOS]).wait()
    for u in range(1 - NS, 1):
        wait_burst(*K, u, -u)
    st0 = {}
    q0 = qproj(0)
    qbuf[...] = qproj(1)
    for c in range(NT):
        qk_tile(st0, q0, 0, c)
    mbuf[...] = row_max(st0)

    def compute(i, q, with_q):
        st = {}
        m = mbuf[...]
        for c in range(NT + SKEW):
            if c < NT:
                pv_tile(st, exp_tile(st, m, c), i, c)
            if c == 0 and with_q:
                q_next = qproj(i + 2)
            if c >= SKEW:
                qk_tile(st, q, i + 1, c - SKEW)
        acc_ref[...] += oproj(onorm(st, inv_sum(st)), i)
        if with_q:
            qbuf[...] = q_next
        mbuf[...] = row_max(st)

        @pl.when(i % H == H - 1)
        def _():
            obuf[i // H] = acc_ref[...].astype(BF)
            acc_ref[...] = jnp.zeros_like(acc_ref)

    def steady_step(i, carry):
        start_pairs(_burst(i + 2, PV0, NP) + _burst(i + 3, 0, PV0),
                    _burst(i + 2, PK0, NP) + _burst(i + 3, 0, PK0))

        @pl.when(i == 0)
        def _():
            for u in range(1 - NS, 0):
                wait_burst(*V, u, -u)

        wait_burst(*K, i + 1)
        wait_burst(*V, i)
        compute(i, qbuf[...], True)
        return carry

    jax.lax.fori_loop(0, W0, steady_step, 0)
    qall[0] = qbuf[...]

    def winddown_step(i, carry):
        def dispatch(lo, hi):
            if hi - lo > 1:
                mid = (lo + hi) // 2
                jax.lax.cond(i < mid, lambda: dispatch(lo, mid), lambda: dispatch(mid, hi))
                return
            if lo == W0:
                start_pairs(_burst(USTAR, PV0, NP), _burst(USTAR, PK0, NP))
            start_plan(lo)
            wait_slab(K, lo + 1)
            wait_slab(V, lo)

        dispatch(W0, I0)
        compute(i, qall[i - W0], False)
        return carry

    jax.lax.fori_loop(W0, I0, winddown_step, 0)

    s0, s1, s2 = {}, {}, {}
    start_plan(I0)
    wait_slab(K, I1)
    wait_slab(V, I0, late=False)
    m0 = mbuf[...]
    q = qall[NQ - 2]
    for c in range(NT):
        p = exp_tile(s0, m0, c)
        if c < TA:
            pv_tile(s0, p, I0, c)
        else:
            p0buf[:, cols(c - TA)] = p
        qk_tile(s1, q, I1, c)
    r0 = inv_sum(s0)
    m1 = row_max(s1)
    wait_slab(V, I0, late=True)
    wait_slab(K, I2)
    q = qall[NQ - 1]
    for c in range(TA, NT):
        pv_tile(s0, p0buf[:, cols(c - TA)], I0, c)
    for c in range(NT):
        p1buf[:, cols(c)] = exp_tile(s1, m1, c)
        qk_tile(s2, q, I2, c)
    acc_ref[...] += oproj(onorm(s0, r0), I0)
    r1 = inv_sum(s1)
    m2 = row_max(s2)
    wait_slab(V, I1)
    for c in range(NT):
        pv_tile(s1, p1buf[:, cols(c)], I1, c)
    o1 = onorm(s1, r1)
    wait_slab(V, I2, late=False)
    o_copy(0, B - 1, OS0).start(priority=LO)
    early = [c for c in range(NT) if not _late(I2, c // TP)]
    acc_ref[...] += oproj(o1, I1)
    for c in early:
        pv_tile(s2, exp_tile(s2, m2, c), I2, c)
    wait_slab(V, I2, late=True)
    for c in range(NT):
        if c not in early:
            pv_tile(s2, exp_tile(s2, m2, c), I2, c)
    obuf[B - 1] = (acc_ref[...] + oproj(onorm(s2, inv_sum(s2)), I2)).astype(BF)
    o_copy(B - 1, 1, OS1).start(priority=HI)
    o_copy(0, B - 1, OS0).wait()
    o_copy(B - 1, 1, OS1).wait()


@jax.jit
def pallas_standalone__mha_block_cached__near_ridge_kernel(
    x: jax.Array,
    k_cache: jax.Array,
    v_cache: jax.Array,
    wq: jax.Array,
    wo: jax.Array,
):
    any_spec = pl.BlockSpec(memory_space=pl.ANY)
    return pl.pallas_call(
        _kernel,
        in_specs=[any_spec] * 5,
        out_specs=any_spec,
        out_shape=jax.ShapeDtypeStruct((B, SQ, D), x.dtype),
        scratch_shapes=[
            pltpu.VMEM((DEPTH, NS, PR, DH), BF),
            pltpu.VMEM((DEPTH, NS, PR, DH), BF),
            pltpu.VMEM((XG, XR, D), BF),
            pltpu.VMEM((WG, WR, H * DH), BF),
            pltpu.VMEM((WG, WR, H * DH), BF),
            pltpu.VMEM((SQ, SK), F32),
            pltpu.VMEM((SQ, T), F32),
            pltpu.VMEM((SQ, DH), BF),
            pltpu.VMEM((NQ, SQ, DH), BF),
            pltpu.VMEM((SQ, D), F32),
            pltpu.VMEM((B, SQ, D), BF),
            pltpu.VMEM((SQ, (NT - TA) * T), BF),
            pltpu.VMEM((SQ, SK), BF),
            pltpu.SemaphoreType.DMA((NSEM,)),
        ],
        compiler_params=pltpu.CompilerParams(
            vmem_limit_bytes=64 * 1024 * 1024,
            disable_bounds_checks=True,
            disable_semaphore_checks=True,
        ),
    )(
        x.reshape(XG, XR, D),
        k_cache.reshape(NSTEP, SK, DH),
        v_cache.reshape(NSTEP, SK, DH),
        wq.reshape(WG, WR, H * DH),
        wo.T.reshape(WG, WR, H * DH),
    )
```
